```python
import os as _os
_os.environ.setdefault('JAX_PLATFORMS', 'cpu')
import jax
import jax.numpy as jnp

def _softmax(x, axis=-1):
    return jax.nn.softmax(x, axis=axis)

def _gelu(x):
    return jax.nn.gelu(x, approximate=True)

def _silu(x):
    return jax.nn.silu(x)

def _sigmoid(x):
    return jax.nn.sigmoid(x)

def _layernorm(x, axis=-1, eps=1e-05):
    m = jnp.mean(x, axis=axis, keepdims=True)
    v = jnp.var(x, axis=axis, keepdims=True)
    return (x - m) / jnp.sqrt(v + eps)

def _scatter_add(tgt, idx, src, axis=0):
    return tgt.at[idx].add(src)

def _segment_sum(src, seg, n):
    return jax.ops.segment_sum(src, seg, n)

class _Rng:

    def __init__(self, key):
        self._k = key

    def _next(self):
        self._k, sub = jax.random.split(self._k)
        return sub

    def normal(self, shape):
        return jax.random.normal(self._next(), shape, dtype=jnp.bfloat16)

    def randint(self, lo, hi, shape):
        return jax.random.randint(self._next(), shape, lo, hi, dtype=jnp.int32)

    def uniform(self, shape, lo=0.0, hi=1.0):
        return jax.random.uniform(self._next(), shape, jnp.bfloat16, lo, hi)

    def permutation(self, n):
        return jax.random.permutation(self._next(), n)
kernel_name = 'adaLN_cond__mha_block_cached__geglu_ffn__prompt'

def setup_inputs():
    _rng = _Rng(jax.random.key(int.from_bytes(__import__("os").urandom(4), "little")))
    _w = lambda a: (lambda t: t.astype(jnp.bfloat16) if jnp.issubdtype(t.dtype, jnp.floating) else t)(jnp.asarray(a))

    def _A_setup():
        B, Sq, D = (1, 2048, 512)
        H, Sk, Dh = (32, 2048, 128)
        return {'x': _w((lambda *s: _rng.normal(s) * 0.05)(B, Sq, D)), 'k_cache': _w((lambda *s: _rng.normal(s) * 3.2)(B, H, Sk, Dh)), 'v_cache': _w((lambda *s: _rng.normal(s) * 0.4)(B, H, Sk, Dh)), 'wq': _w((lambda *s: _rng.normal(s) * 1.6)(D, H * Dh) * D ** (-0.5)), 'wo': _w((lambda *s: _rng.normal(s) * 0.4)(H * Dh, D) * (H * Dh) ** (-0.5))}
    _A_in = _A_setup()

    def _B_setup():
        B, S, D, F = (1, 2048, 512, 1792)
        return {'x': _w((lambda *s: _rng.normal(s) * 0.05)(B, S, D)), 'w_gate': _w((lambda *s: _rng.normal(s) * 0.05)(D, F)), 'w_up': _w((lambda *s: _rng.normal(s) * 0.05)(D, F)), 'w_down': _w((lambda *s: _rng.normal(s) * 0.05)(F, D))}
    _B_in = _B_setup()
    return {'A_x': _A_in['x'], 'A_k_cache': _A_in['k_cache'], 'A_v_cache': _A_in['v_cache'], 'A_wq': _A_in['wq'], 'A_wo': _A_in['wo'], 'B_x': _B_in['x'], 'B_w_gate': _B_in['w_gate'], 'B_w_up': _B_in['w_up'], 'B_w_down': _B_in['w_down'], 'c': _w((lambda *s: _rng.normal(s) * 0.05)(1, 512) * 8.0), 'w_mod': _w((lambda *s: _rng.normal(s) * 0.05)(512, 6 * 512) * 512 ** (-0.5) * 8.0)}

def reference(A_x, A_k_cache, A_v_cache, A_wq, A_wo, B_x, B_w_gate, B_w_up, B_w_down, c, w_mod):

    def _A_ref(x, k_cache, v_cache, wq, wo):
        B, Sq, D = x.shape
        H, Dh = (32, 128)
        q = (lambda x, *d: x.transpose(*d))((x @ wq).reshape(B, Sq, H, Dh), 0, 2, 1, 3)
        scores = jnp.einsum('bhqd,bhkd->bhqk', q, k_cache) * Dh ** (-0.5)
        p = _softmax(scores, axis=-1)
        o = jnp.einsum('bhqk,bhkd->bhqd', p, v_cache)
        return (lambda x, *d: x.transpose(*d))(o, 0, 2, 1, 3).reshape(B, Sq, H * Dh) @ wo

    def _B_ref(x, w_gate, w_up, w_down):
        return _gelu(x @ w_gate) * (x @ w_up) @ w_down
    x = A_x
    mod = (_silu(c) @ w_mod).reshape(c.shape[0], 6, 1, -1)
    sa, ca, ga, sb, cb, gb = (mod[:, 0].copy(), mod[:, 1].copy(), mod[:, 2].copy(), mod[:, 3].copy(), mod[:, 4].copy(), mod[:, 5].copy())
    h = _layernorm(x, axis=-1) * (1 + ca) + sa
    x = x + ga * _A_ref(h, A_k_cache, A_v_cache, A_wq, A_wo)
    h = _layernorm(x, axis=-1) * (1 + cb) + sb
    x = x + gb * _B_ref(h, B_w_gate, B_w_up, B_w_down)
    return x
```

```python
import functools
import math

import jax
import jax.numpy as jnp
from jax import lax
import jax.experimental.pallas as pl
import jax.experimental.pallas.tpu as pltpu

_F32 = jnp.float32
_BF16 = jnp.bfloat16
_LN_EPS = 1e-5


def _layernorm_f32(x):
    m = jnp.mean(x, axis=-1, keepdims=True)
    xc = x - m
    v = jnp.mean(xc * xc, axis=-1, keepdims=True)
    return xc * lax.rsqrt(v + _LN_EPS)


def _fused_block_kernel(
    x_ref,
    k_ref,
    v_ref,
    wq_ref,
    wo_ref,
    wg_ref,
    wu_ref,
    wd_ref,
    c_ref,
    wmod_ref,
    o_ref,
    h_scr,
    acc_scr,
    mod_scr,
    *,
    num_heads: int,
    tq: int,
    tf: int,
):
    head = pl.program_id(0)
    S, D = x_ref.shape
    Dh = k_ref.shape[-1]
    n_q = S // tq

    @pl.when(head == 0)
    def _prologue():
        c = c_ref[...].astype(_F32)
        sc = c * jax.nn.sigmoid(c)
        mod_scr[...] = jnp.dot(sc.astype(_BF16), wmod_ref[...],
                               preferred_element_type=_F32)
        sa = mod_scr[:, 0 * D:1 * D]
        ca = mod_scr[:, 1 * D:2 * D]

        def ln_body(i, carry):
            rows = pl.ds(pl.multiple_of(i * tq, tq), tq)
            xf = x_ref[rows, :].astype(_F32)
            h = _layernorm_f32(xf) * (1.0 + ca) + sa
            h_scr[rows, :] = h.astype(_BF16)
            acc_scr[rows, :] = jnp.zeros((tq, D), _F32)
            return carry

        lax.fori_loop(0, n_q, ln_body, 0)

    q_scale = (Dh ** -0.5) * math.log2(math.e)

    def attn_body(i, carry):
        rows = pl.ds(pl.multiple_of(i * tq, tq), tq)
        q = jnp.dot(h_scr[rows, :], wq_ref[...], preferred_element_type=_F32)
        q = (q * q_scale).astype(_BF16)
        s = lax.dot_general(q, k_ref[...], (((1,), (1,)), ((), ())),
                            preferred_element_type=_F32)
        m = jnp.max(s, axis=-1, keepdims=True)
        p = jnp.exp2(s - m)
        l = jnp.sum(p, axis=-1, keepdims=True)
        o = jnp.dot(p.astype(_BF16), v_ref[...], preferred_element_type=_F32)
        o = o / l
        acc_scr[rows, :] += jnp.dot(o.astype(_BF16), wo_ref[...],
                                    preferred_element_type=_F32)
        return carry

    lax.fori_loop(0, n_q, attn_body, 0, unroll=2)

    @pl.when(head == num_heads - 1)
    def _epilogue():
        ga = mod_scr[:, 2 * D:3 * D]
        sb = mod_scr[:, 3 * D:4 * D]
        cb = mod_scr[:, 4 * D:5 * D]
        gb = mod_scr[:, 5 * D:6 * D]

        def ffn_body(i, carry):
            rows = pl.ds(pl.multiple_of(i * tf, tf), tf)
            x1 = x_ref[rows, :].astype(_F32) + ga * acc_scr[rows, :]
            h2 = (_layernorm_f32(x1) * (1.0 + cb) + sb).astype(_BF16)
            g = jnp.dot(h2, wg_ref[...], preferred_element_type=_F32)
            u = jnp.dot(h2, wu_ref[...], preferred_element_type=_F32)
            a = jax.nn.gelu(g, approximate=True) * u
            y = jnp.dot(a.astype(_BF16), wd_ref[...], preferred_element_type=_F32)
            o_ref[rows, :] = (x1 + gb * y).astype(o_ref.dtype)
            return carry

        lax.fori_loop(0, S // tf, ffn_body, 0)


@jax.jit
def pallas_adaLN_cond__mha_block_cached__geglu_ffn__prompt_kernel(
    A_x: jax.Array,
    A_k_cache: jax.Array,
    A_v_cache: jax.Array,
    A_wq: jax.Array,
    A_wo: jax.Array,
    B_x: jax.Array,
    B_w_gate: jax.Array,
    B_w_up: jax.Array,
    B_w_down: jax.Array,
    c: jax.Array,
    w_mod: jax.Array,
):
    del B_x
    B, S, D = A_x.shape
    _, H, Sk, Dh = A_k_cache.shape
    F = B_w_gate.shape[1]
    assert B == 1 and A_wq.shape == (D, H * Dh) and A_wo.shape == (H * Dh, D)

    tq = 256
    tf = 256

    kernel = functools.partial(_fused_block_kernel, num_heads=H, tq=tq, tf=tf)

    const2 = lambda h: (0, 0)
    out = pl.pallas_call(
        kernel,
        grid=(H,),
        in_specs=[
            pl.BlockSpec((None, S, D), lambda h: (0, 0, 0)),
            pl.BlockSpec((None, None, Sk, Dh), lambda h: (0, h, 0, 0)),
            pl.BlockSpec((None, None, Sk, Dh), lambda h: (0, h, 0, 0)),
            pl.BlockSpec((D, Dh), lambda h: (0, h)),
            pl.BlockSpec((Dh, D), lambda h: (h, 0)),
            pl.BlockSpec((D, F), const2),
            pl.BlockSpec((D, F), const2),
            pl.BlockSpec((F, D), const2),
            pl.BlockSpec((1, D), const2),
            pl.BlockSpec((D, 6 * D), const2),
        ],
        out_specs=pl.BlockSpec((None, S, D), lambda h: (0, 0, 0)),
        out_shape=jax.ShapeDtypeStruct((B, S, D), A_x.dtype),
        scratch_shapes=[
            pltpu.VMEM((S, D), _BF16),
            pltpu.VMEM((S, D), _F32),
            pltpu.VMEM((1, 6 * D), _F32),
        ],
        compiler_params=pltpu.CompilerParams(
            dimension_semantics=("arbitrary",),
            vmem_limit_bytes=100 * 1024 * 1024,
        ),
        name="adaln_mha_geglu_block",
    )(A_x, A_k_cache, A_v_cache, A_wq, A_wo, B_w_gate, B_w_up, B_w_down, c, w_mod)
    return out
```

```python
import functools
import math

import jax
import jax.numpy as jnp
from jax import lax
import jax.experimental.pallas as pl
import jax.experimental.pallas.tpu as pltpu

_F32 = jnp.float32
_BF16 = jnp.bfloat16
_LN_EPS = 1e-5


def _layernorm_f32(x):
    m = jnp.mean(x, axis=-1, keepdims=True)
    xc = x - m
    v = jnp.mean(xc * xc, axis=-1, keepdims=True)
    return xc * lax.rsqrt(v + _LN_EPS)


def _fused_block_kernel(
    x_ref,
    k_ref,
    v_ref,
    wq_ref,
    wo_ref,
    wg_hbm,
    wu_hbm,
    wd_hbm,
    c_ref,
    wmod_ref,
    o_hbm,
    h_scr,
    acc_scr,
    mod_scr,
    p0_scr,
    p1_scr,
    wg_scr,
    wu_scr,
    wd_scr,
    w_sems,
    o_sems,
    *,
    num_heads: int,
    tq: int,
    tf: int,
    strip: int,
):
    head = pl.program_id(0)
    S, D = x_ref.shape
    Sk, Dh = k_ref.shape
    n_q = S // tq
    n_mod_steps = 6 * D // wmod_ref.shape[1]

    def ffn_weight_copies():
        return [
            pltpu.make_async_copy(src, dst, w_sems.at[i])
            for i, (src, dst) in enumerate(
                ((wg_hbm, wg_scr), (wu_hbm, wu_scr), (wd_hbm, wd_scr)))
        ]

    for t in range(n_mod_steps):
        @pl.when(head == t)
        def _modulation(t=t):
            c = c_ref[...].astype(_F32)
            sc = c * jax.nn.sigmoid(c)
            w = wmod_ref.shape[1]
            mod_scr[:, t * w:(t + 1) * w] = jnp.dot(
                sc.astype(_BF16), wmod_ref[...], preferred_element_type=_F32)

    @pl.when(head == 0)
    def _prologue():
        for cp in ffn_weight_copies():
            cp.start()
        sa = mod_scr[:, 0 * D:1 * D]
        ca = mod_scr[:, 1 * D:2 * D]

        def ln_body(i, carry):
            rows = pl.ds(pl.multiple_of(i * tq, tq), tq)
            xf = x_ref[rows, :].astype(_F32)
            h = _layernorm_f32(xf) * (1.0 + ca) + sa
            h_scr[rows, :] = h.astype(_BF16)
            acc_scr[rows, :] = jnp.zeros((tq, D), _F32)
            return carry

        lax.fori_loop(0, n_q, ln_body, 0)

    q_scale = (Dh ** -0.5) * math.log2(math.e)

    def scores(rows):
        q = jnp.dot(h_scr[rows, :], wq_ref[...], preferred_element_type=_F32)
        q = (q * q_scale).astype(_BF16)
        return lax.dot_general(q, k_ref[...], (((1,), (1,)), ((), ())),
                               preferred_element_type=_F32)

    def finish(rows, s, p_scr):
        m = jnp.max(s, axis=-1, keepdims=True)
        ls = []
        for r in range(0, tq, strip):
            e = jnp.exp2(s[r:r + strip, :] - m[r:r + strip, :])
            ls.append(jnp.sum(e, axis=-1, keepdims=True))
            p_scr[r // 2:(r + strip) // 2, :] = pltpu.bitcast(e.astype(_BF16), jnp.uint32)
        l = jnp.concatenate(ls, axis=0)
        p = pltpu.bitcast(p_scr[...], _BF16)
        o = jnp.dot(p, v_ref[...], preferred_element_type=_F32)
        o = o / l
        acc_scr[rows, :] += jnp.dot(o.astype(_BF16), wo_ref[...],
                                    preferred_element_type=_F32)

    p_bufs = (p0_scr, p1_scr)
    row_sl = [pl.ds(j * tq, tq) for j in range(n_q)]
    s_next = scores(row_sl[0])
    for j in range(n_q):
        s_cur = s_next
        if j + 1 < n_q:
            s_next = scores(row_sl[j + 1])
        finish(row_sl[j], s_cur, p_bufs[j % 2])

    @pl.when(head == num_heads - 1)
    def _epilogue():
        for cp in ffn_weight_copies():
            cp.wait()
        ga = mod_scr[:, 2 * D:3 * D]
        sb = mod_scr[:, 3 * D:4 * D]
        cb = mod_scr[:, 4 * D:5 * D]
        gb = mod_scr[:, 5 * D:6 * D]

        n_f = S // tf

        def out_copy(i):
            rows = pl.ds(pl.multiple_of(i * tf, tf), tf)
            return pltpu.make_async_copy(h_scr.at[rows, :], o_hbm.at[rows, :],
                                         o_sems.at[i])

        def ffn_body(i, carry):
            rows = pl.ds(pl.multiple_of(i * tf, tf), tf)
            x1 = x_ref[rows, :].astype(_F32) + ga * acc_scr[rows, :]
            h2 = (_layernorm_f32(x1) * (1.0 + cb) + sb).astype(_BF16)
            g = jnp.dot(h2, wg_scr[...], preferred_element_type=_F32)
            u = jnp.dot(h2, wu_scr[...], preferred_element_type=_F32)
            a = jax.nn.gelu(g, approximate=True) * u
            y = jnp.dot(a.astype(_BF16), wd_scr[...], preferred_element_type=_F32)
            h_scr[rows, :] = (x1 + gb * y).astype(h_scr.dtype)
            out_copy(i).start()
            return carry

        lax.fori_loop(0, n_f, ffn_body, 0, unroll=2)

        def wait_body(i, carry):
            out_copy(i).wait()
            return carry

        lax.fori_loop(0, n_f, wait_body, 0)


@jax.jit
def pallas_adaLN_cond__mha_block_cached__geglu_ffn__prompt_kernel(
    A_x: jax.Array,
    A_k_cache: jax.Array,
    A_v_cache: jax.Array,
    A_wq: jax.Array,
    A_wo: jax.Array,
    B_x: jax.Array,
    B_w_gate: jax.Array,
    B_w_up: jax.Array,
    B_w_down: jax.Array,
    c: jax.Array,
    w_mod: jax.Array,
):
    del B_x
    B, S, D = A_x.shape
    _, H, Sk, Dh = A_k_cache.shape
    F = B_w_gate.shape[1]
    assert B == 1 and A_wq.shape == (D, H * Dh) and A_wo.shape == (H * Dh, D)
    n_mod_steps = 3
    assert H >= n_mod_steps

    tq = 256
    tf = 256
    strip = 32

    kernel = functools.partial(_fused_block_kernel, num_heads=H, tq=tq, tf=tf, strip=strip)

    const2 = lambda h: (0, 0)
    out = pl.pallas_call(
        kernel,
        grid=(H,),
        in_specs=[
            pl.BlockSpec((None, S, D), lambda h: (0, 0, 0)),
            pl.BlockSpec((None, None, Sk, Dh), lambda h: (0, h, 0, 0)),
            pl.BlockSpec((None, None, Sk, Dh), lambda h: (0, h, 0, 0)),
            pl.BlockSpec((D, Dh), lambda h: (0, h)),
            pl.BlockSpec((Dh, D), lambda h: (h, 0)),
            pl.BlockSpec(memory_space=pl.ANY),
            pl.BlockSpec(memory_space=pl.ANY),
            pl.BlockSpec(memory_space=pl.ANY),
            pl.BlockSpec((1, D), const2),
            pl.BlockSpec((D, 6 * D // n_mod_steps),
                         lambda h: (0, jnp.minimum(h, n_mod_steps - 1))),
        ],
        out_specs=pl.BlockSpec(memory_space=pl.ANY),
        out_shape=jax.ShapeDtypeStruct((S, D), A_x.dtype),
        scratch_shapes=[
            pltpu.VMEM((S, D), _BF16),
            pltpu.VMEM((S, D), _F32),
            pltpu.VMEM((1, 6 * D), _F32),
            pltpu.VMEM((tq // 2, Sk), jnp.uint32),
            pltpu.VMEM((tq // 2, Sk), jnp.uint32),
            pltpu.VMEM((D, F), _BF16),
            pltpu.VMEM((D, F), _BF16),
            pltpu.VMEM((D, F)[::-1], _BF16),
            pltpu.SemaphoreType.DMA((3,)),
            pltpu.SemaphoreType.DMA((S // tf,)),
        ],
        compiler_params=pltpu.CompilerParams(
            dimension_semantics=("arbitrary",),
            vmem_limit_bytes=100 * 1024 * 1024,
        ),
        name="adaln_mha_geglu_block",
    )(A_x, A_k_cache, A_v_cache, A_wq, A_wo, B_w_gate, B_w_up, B_w_down, c, w_mod)
    return out.reshape(B, S, D)
```

```python
import functools
import math

import jax
import jax.numpy as jnp
from jax import lax
import jax.experimental.pallas as pl
import jax.experimental.pallas.tpu as pltpu

_F32 = jnp.float32
_BF16 = jnp.bfloat16
_LN_EPS = 1e-5


def _layernorm_f32(x):
    m = jnp.mean(x, axis=-1, keepdims=True)
    xc = x - m
    v = jnp.mean(xc * xc, axis=-1, keepdims=True)
    return xc * lax.rsqrt(v + _LN_EPS)


def _fused_block_kernel(
    x_ref,
    k_ref,
    v_ref,
    wq_ref,
    wo_ref,
    wg_hbm,
    wu_hbm,
    wd_hbm,
    c_ref,
    wmod_ref,
    o_hbm,
    h_scr,
    acc_scr,
    mod_scr,
    p0_scr,
    p1_scr,
    wg_scr,
    wu_scr,
    wd_scr,
    w_sems,
    o_sems,
    *,
    num_heads: int,
    tq: int,
    tf: int,
    strip: int,
):
    head = pl.program_id(0)
    S, D = x_ref.shape
    Sk, Dh = k_ref.shape
    n_q = S // tq
    n_mod_steps = 6 * D // wmod_ref.shape[1]

    def ffn_weight_copies():
        return [
            pltpu.make_async_copy(src, dst, w_sems.at[i])
            for i, (src, dst) in enumerate(
                ((wg_hbm, wg_scr), (wu_hbm, wu_scr), (wd_hbm, wd_scr)))
        ]

    for t in range(n_mod_steps):
        @pl.when(head == t)
        def _modulation(t=t):
            c = c_ref[...].astype(_F32)
            sc = c * jax.nn.sigmoid(c)
            w = wmod_ref.shape[1]
            mod_scr[:, t * w:(t + 1) * w] = jnp.dot(
                sc.astype(_BF16), wmod_ref[...], preferred_element_type=_F32)

    @pl.when(head == 0)
    def _prologue():
        for cp in ffn_weight_copies():
            cp.start()
        sa = mod_scr[:, 0 * D:1 * D]
        ca = mod_scr[:, 1 * D:2 * D]

        def ln_body(i, carry):
            rows = pl.ds(pl.multiple_of(i * tq, tq), tq)
            xf = x_ref[rows, :].astype(_F32)
            h = _layernorm_f32(xf) * (1.0 + ca) + sa
            h_scr[rows, :] = h.astype(_BF16)
            acc_scr[rows, :] = jnp.zeros((tq, D), _F32)
            return carry

        lax.fori_loop(0, n_q, ln_body, 0)

    q_scale = (Dh ** -0.5) * math.log2(math.e)

    n_chunks = 4
    kc = Sk // n_chunks
    n_strips = tq // strip
    spc = n_strips // n_chunks

    def score_chunks(rows):
        q = jnp.dot(h_scr[rows, :], wq_ref[...], preferred_element_type=_F32)
        q = (q * q_scale).astype(_BF16)
        return [lax.dot_general(q, k_ref[c * kc:(c + 1) * kc, :], (((1,), (1,)), ((), ())),
                                preferred_element_type=_F32) for c in range(n_chunks)]

    def finish(rows, s, p_scr, gates):
        m = jnp.max(s, axis=-1, keepdims=True)
        ls = []
        for t in range(n_strips):
            r = t * strip
            mt = m[r:r + strip, :]
            if gates is not None and t >= spc:
                mt = mt + jnp.nan_to_num(gates[t // spc][r:r + strip, 0:1]) * 0.0
            e = jnp.exp2(s[r:r + strip, :] - mt)
            ls.append(jnp.sum(e, axis=-1, keepdims=True))
            p_scr[r // 2:(r + strip) // 2, :] = pltpu.bitcast(e.astype(_BF16), jnp.uint32)
        l = jnp.concatenate(ls, axis=0)
        p = pltpu.bitcast(p_scr[...], _BF16)
        o = jnp.dot(p, v_ref[...], preferred_element_type=_F32)
        o = o / l
        acc_scr[rows, :] += jnp.dot(o.astype(_BF16), wo_ref[...],
                                    preferred_element_type=_F32)

    p_bufs = (p0_scr, p1_scr)
    row_sl = [pl.ds(j * tq, tq) for j in range(n_q)]
    s_next = score_chunks(row_sl[0])
    for j in range(n_q):
        s_cur = jnp.concatenate(s_next, axis=1)
        s_next = score_chunks(row_sl[j + 1]) if j + 1 < n_q else None
        finish(row_sl[j], s_cur, p_bufs[j % 2], s_next)

    @pl.when(head == num_heads - 1)
    def _epilogue():
        for cp in ffn_weight_copies():
            cp.wait()
        ga = mod_scr[:, 2 * D:3 * D]
        sb = mod_scr[:, 3 * D:4 * D]
        cb = mod_scr[:, 4 * D:5 * D]
        gb = mod_scr[:, 5 * D:6 * D]

        n_f = S // tf

        def out_copy(i):
            rows = pl.ds(pl.multiple_of(i * tf, tf), tf)
            return pltpu.make_async_copy(h_scr.at[rows, :], o_hbm.at[rows, :],
                                         o_sems.at[i])

        def ffn_body(i, carry):
            rows = pl.ds(pl.multiple_of(i * tf, tf), tf)
            x1 = x_ref[rows, :].astype(_F32) + ga * acc_scr[rows, :]
            h2 = (_layernorm_f32(x1) * (1.0 + cb) + sb).astype(_BF16)
            g = jnp.dot(h2, wg_scr[...], preferred_element_type=_F32)
            u = jnp.dot(h2, wu_scr[...], preferred_element_type=_F32)
            a = jax.nn.gelu(g, approximate=True) * u
            y = jnp.dot(a.astype(_BF16), wd_scr[...], preferred_element_type=_F32)
            h_scr[rows, :] = (x1 + gb * y).astype(h_scr.dtype)
            out_copy(i).start()
            return carry

        lax.fori_loop(0, n_f, ffn_body, 0, unroll=2)

        def wait_body(i, carry):
            out_copy(i).wait()
            return carry

        lax.fori_loop(0, n_f, wait_body, 0)


@jax.jit
def pallas_adaLN_cond__mha_block_cached__geglu_ffn__prompt_kernel(
    A_x: jax.Array,
    A_k_cache: jax.Array,
    A_v_cache: jax.Array,
    A_wq: jax.Array,
    A_wo: jax.Array,
    B_x: jax.Array,
    B_w_gate: jax.Array,
    B_w_up: jax.Array,
    B_w_down: jax.Array,
    c: jax.Array,
    w_mod: jax.Array,
):
    del B_x
    B, S, D = A_x.shape
    _, H, Sk, Dh = A_k_cache.shape
    F = B_w_gate.shape[1]
    assert B == 1 and A_wq.shape == (D, H * Dh) and A_wo.shape == (H * Dh, D)
    n_mod_steps = 3
    assert H >= n_mod_steps

    tq = 256
    tf = 256
    strip = 32

    kernel = functools.partial(_fused_block_kernel, num_heads=H, tq=tq, tf=tf, strip=strip)

    const2 = lambda h: (0, 0)
    out = pl.pallas_call(
        kernel,
        grid=(H,),
        in_specs=[
            pl.BlockSpec((None, S, D), lambda h: (0, 0, 0)),
            pl.BlockSpec((None, None, Sk, Dh), lambda h: (0, h, 0, 0)),
            pl.BlockSpec((None, None, Sk, Dh), lambda h: (0, h, 0, 0)),
            pl.BlockSpec((D, Dh), lambda h: (0, h)),
            pl.BlockSpec((Dh, D), lambda h: (h, 0)),
            pl.BlockSpec(memory_space=pl.ANY),
            pl.BlockSpec(memory_space=pl.ANY),
            pl.BlockSpec(memory_space=pl.ANY),
            pl.BlockSpec((1, D), const2),
            pl.BlockSpec((D, 6 * D // n_mod_steps),
                         lambda h: (0, jnp.minimum(h, n_mod_steps - 1))),
        ],
        out_specs=pl.BlockSpec(memory_space=pl.ANY),
        out_shape=jax.ShapeDtypeStruct((S, D), A_x.dtype),
        scratch_shapes=[
            pltpu.VMEM((S, D), _BF16),
            pltpu.VMEM((S, D), _F32),
            pltpu.VMEM((1, 6 * D), _F32),
            pltpu.VMEM((tq // 2, Sk), jnp.uint32),
            pltpu.VMEM((tq // 2, Sk), jnp.uint32),
            pltpu.VMEM((D, F), _BF16),
            pltpu.VMEM((D, F), _BF16),
            pltpu.VMEM((D, F)[::-1], _BF16),
            pltpu.SemaphoreType.DMA((3,)),
            pltpu.SemaphoreType.DMA((S // tf,)),
        ],
        compiler_params=pltpu.CompilerParams(
            dimension_semantics=("arbitrary",),
            vmem_limit_bytes=100 * 1024 * 1024,
        ),
        name="adaln_mha_geglu_block",
    )(A_x, A_k_cache, A_v_cache, A_wq, A_wo, B_w_gate, B_w_up, B_w_down, c, w_mod)
    return out.reshape(B, S, D)
```
